```python
import jax
import jax.numpy as jnp

def _softmax(x, axis=-1):
    return jax.nn.softmax(x, axis=axis)
def _gelu(x):
    return jax.nn.gelu(x, approximate=True)
def _silu(x):
    return jax.nn.silu(x)
def _sigmoid(x):
    return jax.nn.sigmoid(x)
def _layernorm(x, axis=-1, eps=1e-5):
    m = jnp.mean(x, axis=axis, keepdims=True)
    v = jnp.var(x, axis=axis, keepdims=True)
    return (x - m) / jnp.sqrt(v + eps)
def _scatter_add(tgt, idx, src, axis=0):
    return tgt.at[idx].add(src)
def _segment_sum(src, seg, n):
    return jax.ops.segment_sum(src, seg, n)
class _Rng:
    def __init__(self, key):
        self._k = key
    def _next(self):
        self._k, sub = jax.random.split(self._k)
        return sub
    def normal(self, shape):
        return jax.random.normal(self._next(), shape, dtype=jnp.bfloat16)
    def randint(self, lo, hi, shape):
        return jax.random.randint(self._next(), shape, lo, hi, dtype=jnp.int32)
    def uniform(self, shape, lo=0.0, hi=1.0):
        return jax.random.uniform(self._next(), shape, jnp.bfloat16, lo, hi)
    def permutation(self, n):
        return jax.random.permutation(self._next(), n)


kernel_name = 'standalone__instancenorm__prompt'

def setup_inputs():
    _rng = _Rng(jax.random.key(int.from_bytes(__import__("os").urandom(4), "little")))
    _w = (lambda a: (lambda t: t.astype(jnp.bfloat16) if jnp.issubdtype(t.dtype, jnp.floating) else t)(jnp.asarray(a)))
    B, C, H, W = 2, 1024, 2048, 32
    return {
        "x": _w((lambda *s: _rng.normal(s) * 0.05)(B, C, H, W)),
        "g": _w((lambda *s: _rng.normal(s) * 0.05)(C) + 1.0),
        "b": _w((lambda *s: _rng.normal(s) * 0.05)(C)),
    }

def reference(x, g, b):
    mu = x.mean(axis=(-2, -1), keepdims=True)
    var = ((x - mu) * (x - mu)).mean(axis=(-2, -1), keepdims=True)
    xhat = (x - mu) / jnp.sqrt(var + 1e-5)
    return xhat * g.reshape(1, -1, 1, 1) + b.reshape(1, -1, 1, 1)
```

```python
import functools

import jax
import jax.numpy as jnp
from jax import lax
import jax.experimental.pallas as pl
import jax.experimental.pallas.tpu as pltpu

_EPS = 1e-5
_R = 8
_P = 64
_D = 2
_LANES = 128
_SUB = 8


def _vreg_sum(tiles):
    while len(tiles) > 1:
        tiles = [tiles[i] + tiles[i + 1] for i in range(0, len(tiles), 2)]
    return tiles[0]


def _kernel(x_hbm, g_ref, b_ref, o_hbm, buf, part, mu_s, sc_s, bb_s, gb_v, gb_s,
            sems, gb_sem, *, n_inst, n_ch, rows, cols):
    R, P, D = _R, _P, _D
    n_chunks = n_inst // R
    n_ops = 2 * n_chunks
    inv_n = 1.0 / (rows * cols)
    n_col = cols // _LANES
    n_row = rows // _SUB
    g_rows = n_ch // _LANES

    def rd(c, slot):
        return pltpu.make_async_copy(
            x_hbm.at[pl.ds(c * R, R)], buf.at[pl.ds(slot * R, R)], sems.at[slot])

    def wr(c, slot):
        return pltpu.make_async_copy(
            buf.at[pl.ds(slot * R, R)], o_hbm.at[pl.ds(c * R, R)], sems.at[slot])

    for s in range(D):
        rd(s, s).start()

    gb_v[0:g_rows, :] = g_ref[...].astype(jnp.float32)
    gb_v[g_rows:2 * g_rows, :] = b_ref[...].astype(jnp.float32)
    gb_copy = pltpu.make_async_copy(gb_v, gb_s, gb_sem)
    gb_copy.start()
    gb_copy.wait()

    def tile_rows(v):
        return jnp.concatenate([v] * n_row, axis=0)

    def fold_rows(v):
        return _vreg_sum([v[i * _SUB:(i + 1) * _SUB] for i in range(n_row)])

    def total(p):
        return jnp.sum(jnp.sum(p, axis=2, keepdims=True), axis=1, keepdims=True)

    def stats(c, slot):
        base = slot * R

        def sum_pass(r, carry):
            xv = fold_rows(buf[base + r].astype(jnp.float32))
            part[r] = _vreg_sum(
                [xv[:, j * _LANES:(j + 1) * _LANES] for j in range(n_col)])
            return carry

        lax.fori_loop(0, R, sum_pass, 0)
        mu_s[pl.ds(base, R)] = jnp.broadcast_to(
            total(part[...]) * inv_n, (R, _SUB, _LANES))

        def var_pass(r, carry):
            mu = tile_rows(mu_s[base + r])
            xv = buf[base + r].astype(jnp.float32)
            acc = None
            for j in range(n_col):
                d = xv[:, j * _LANES:(j + 1) * _LANES] - mu
                acc = d * d if acc is None else acc + d * d
            part[r] = fold_rows(acc)
            return carry

        lax.fori_loop(0, R, var_pass, 0)
        rstd = jnp.broadcast_to(
            lax.rsqrt(total(part[...]) * inv_n + _EPS), (R, _SUB, _LANES))
        ch0 = lax.rem(c * R, n_ch)
        row = ch0 // _LANES
        col = lax.rem(ch0, _LANES)
        for r in range(R):
            sc_s[base + r] = rstd[r] * gb_s[row, col + r]
            bb_s[base + r] = jnp.full(
                (_SUB, _LANES), gb_s[g_rows + row, col + r], jnp.float32)

    def normalise(slot):
        base = slot * R

        def norm_pass(r, carry):
            mu = tile_rows(mu_s[base + r])
            sc = tile_rows(sc_s[base + r])
            bb = tile_rows(bb_s[base + r])
            for j in range(n_col):
                sl = slice(j * _LANES, (j + 1) * _LANES)
                xv = buf[base + r, :, sl].astype(jnp.float32)
                buf[base + r, :, sl] = ((xv - mu) * sc + bb).astype(buf.dtype)
            return carry

        lax.fori_loop(0, R, norm_pass, 0)

    def decode(t):
        phase = t // P
        slot = t - phase * P
        group = phase // 2
        return phase - 2 * group, group * P + slot, slot

    def body(t, carry):
        t_wr, c, slot = decode(t)
        u = t + D
        u_wr, uc, uslot = decode(u)
        u_rd_ok = jnp.logical_and(u_wr == 0, u < n_ops)
        u_wr_ok = jnp.logical_and(u_wr == 1, u < n_ops)

        @pl.when(u_wr_ok)
        def _():
            normalise(uslot)

        @pl.when(t_wr == 0)
        def _():
            rd(c, slot).wait()

        @pl.when(t_wr == 1)
        def _():
            wr(c, slot).wait()

        @pl.when(u_rd_ok)
        def _():
            rd(uc, uslot).start()

        @pl.when(u_wr_ok)
        def _():
            wr(uc, uslot).start()

        @pl.when(t_wr == 0)
        def _():
            stats(c, slot)

        return carry

    lax.fori_loop(0, n_ops, body, 0)


@jax.jit
def pallas_standalone__instancenorm__prompt_kernel(
    x: jax.Array,
    g: jax.Array,
    b: jax.Array,
):
    B, C, H, W = x.shape
    n_inst = B * C
    xt = jnp.transpose(x, (0, 1, 3, 2)).reshape(n_inst, W, H)
    f32 = jnp.float32
    n_res = _R * _P
    out = pl.pallas_call(
        functools.partial(_kernel, n_inst=n_inst, n_ch=C, rows=W, cols=H),
        in_specs=[
            pl.BlockSpec(memory_space=pl.ANY),
            pl.BlockSpec(memory_space=pltpu.VMEM),
            pl.BlockSpec(memory_space=pltpu.VMEM),
        ],
        out_specs=pl.BlockSpec(memory_space=pl.ANY),
        out_shape=jax.ShapeDtypeStruct((n_inst, W, H), x.dtype),
        scratch_shapes=[
            pltpu.VMEM((n_res, W, H), x.dtype),
            pltpu.VMEM((_R, _SUB, _LANES), f32),
            pltpu.VMEM((n_res, _SUB, _LANES), f32),
            pltpu.VMEM((n_res, _SUB, _LANES), f32),
            pltpu.VMEM((n_res, _SUB, _LANES), f32),
            pltpu.VMEM((2 * C // _LANES, _LANES), f32),
            pltpu.SMEM((2 * C // _LANES, _LANES), f32),
            pltpu.SemaphoreType.DMA((_P,)),
            pltpu.SemaphoreType.DMA,
        ],
        compiler_params=pltpu.CompilerParams(vmem_limit_bytes=100 * 1024 * 1024),
    )(xt, g.reshape(C // _LANES, _LANES), b.reshape(C // _LANES, _LANES))
    return jnp.transpose(out.reshape(B, C, W, H), (0, 1, 3, 2))
```

```python
import functools

import jax
import jax.numpy as jnp
from jax import lax
import jax.experimental.pallas as pl
import jax.experimental.pallas.tpu as pltpu

_EPS = 1e-5
_LANES = 128
_SUB = 8
_TILE = 16
_R = 16
_G = 4
_Q = 8
_SPLIT = 4
_RSUB = 2
_D = 2
_MAX_BURST = 44


def _bursts(n_ops):
    groups = n_ops // _G
    k = -(-n_ops // _MAX_BURST)
    return tuple((groups // k + (i < groups % k)) * _G for i in range(k))


def _pair_sum(tiles):
    while len(tiles) > 1:
        tiles = [tiles[i] + tiles[i + 1] for i in range(0, len(tiles), 2)]
    return tiles[0]


def _kernel(x_hbm, g_hbm, b_hbm, o_hbm, buf, part, mu_s, sc_s, bb_s, gb_in, gb_v,
            gb_s, sems, gb_sems, *, bursts, n_ch, rows, cols):
    R, G, D = _R, _G, _D
    tpi = rows // _TILE
    ipl = _Q // tpi
    lead = R // ipl
    span = G * lead
    q_op = _Q // G
    cw = cols // _SPLIT
    n_col = cols // _LANES
    n_steps = 2 * sum(bursts)
    inv_n = 1.0 / (rows * cols)
    g_rows = n_ch // _LANES

    def rd(c, slot):
        h = lead // _RSUB
        return [
            pltpu.make_async_copy(x_hbm.at[pl.ds(c * lead + i * h, h)],
                                  buf.at[pl.ds(slot * lead + i * h, h)],
                                  sems.at[slot])
            for i in range(_RSUB)
        ]

    def wr(c, slot):
        grp = slot // G
        j = slot - grp * G
        vb = grp * span
        hb = ((c - j) // G) * span
        copies = []
        for qi in range(q_op):
            q = j * q_op + qi
            for s in range(_SPLIT):
                col = pl.ds(s * cw, cw)
                copies.append(pltpu.make_async_copy(
                    buf.at[pl.ds(vb, span), q, :, col],
                    o_hbm.at[pl.ds(hb, span), q, :, col],
                    sems.at[slot]))
        return copies

    def rd_start(c, slot):
        for i, cp in enumerate(rd(c, slot)):
            cp.start(priority=i % 2)

    def wr_start(c, slot):
        for cp in wr(c, slot):
            cp.start()

    def wait_all(copies):
        for cp in copies:
            cp.wait()

    for s in range(D):
        rd_start(s, s)

    gb_copies = [pltpu.make_async_copy(g_hbm, gb_in.at[0], gb_sems.at[0]),
                 pltpu.make_async_copy(b_hbm, gb_in.at[1], gb_sems.at[1])]
    for cp in gb_copies:
        cp.start()
    wait_all(gb_copies)
    gb_v[0:g_rows, :] = gb_in[0].astype(jnp.float32)
    gb_v[g_rows:2 * g_rows, :] = gb_in[1].astype(jnp.float32)
    to_smem = pltpu.make_async_copy(gb_v, gb_s, gb_sems.at[0])
    to_smem.start()
    to_smem.wait()

    def where(slot, r, h):
        return slot * lead + r // ipl, lax.rem(r, ipl) * tpi + h

    def total(p):
        return jnp.sum(jnp.sum(p, axis=2, keepdims=True), axis=1, keepdims=True)

    def twice(v):
        return jnp.concatenate([v, v], axis=0)

    def stats(c, slot):
        base = slot * R

        def sum_pass(r, carry):
            tiles = []
            for h in range(tpi):
                a, q = where(slot, r, h)
                v = buf[a, q].astype(jnp.float32)
                v = v[0:_SUB] + v[_SUB:_TILE]
                tiles += [v[:, j * _LANES:(j + 1) * _LANES] for j in range(n_col)]
            part[r] = _pair_sum(tiles)
            return carry

        lax.fori_loop(0, R, sum_pass, 0)
        mu_s[pl.ds(base, R)] = jnp.broadcast_to(
            total(part[...]) * inv_n, (R, _SUB, _LANES))

        def var_pass(r, carry):
            mu = twice(mu_s[base + r])
            accs = []
            for h in range(tpi):
                a, q = where(slot, r, h)
                v = buf[a, q].astype(jnp.float32)
                acc = None
                for j in range(n_col):
                    d = v[:, j * _LANES:(j + 1) * _LANES] - mu
                    acc = d * d if acc is None else acc + d * d
                accs.append(acc)
            acc = _pair_sum(accs)
            part[r] = acc[0:_SUB] + acc[_SUB:_TILE]
            return carry

        lax.fori_loop(0, R, var_pass, 0)
        rstd = jnp.broadcast_to(
            lax.rsqrt(total(part[...]) * inv_n + _EPS), (R, _SUB, _LANES))
        ch0 = lax.rem(c * R, n_ch)
        row = ch0 // _LANES
        col = lax.rem(ch0, _LANES)
        for r in range(R):
            sc_s[base + r] = rstd[r] * gb_s[row, col + r]
            bb_s[base + r] = jnp.full(
                (_SUB, _LANES), gb_s[g_rows + row, col + r], jnp.float32)

    def normalise(slot):
        base = slot * R

        def norm_pass(r, carry):
            mu = twice(mu_s[base + r])
            sc = twice(sc_s[base + r])
            bb = twice(bb_s[base + r])
            for h in range(tpi):
                a, q = where(slot, r, h)
                for j in range(n_col):
                    sl = slice(j * _LANES, (j + 1) * _LANES)
                    v = buf[a, q, :, sl].astype(jnp.float32)
                    buf[a, q, :, sl] = ((v - mu) * sc + bb).astype(buf.dtype)
            return carry

        lax.fori_loop(0, R, norm_pass, 0)

    def decode(t):
        start, first, size = jnp.int32(0), jnp.int32(0), jnp.int32(bursts[0])
        done = 0
        for prev, cur in zip(bursts[:-1], bursts[1:]):
            done += prev
            hit = t >= 2 * done
            start = jnp.where(hit, 2 * done, start)
            first = jnp.where(hit, done, first)
            size = jnp.where(hit, cur, size)
        w = t - start
        is_wr = w >= size
        slot = jnp.where(is_wr, w - size, w)
        return is_wr, first + slot, slot

    def body(t, carry):
        t_wr, c, slot = decode(t)
        u = t + D
        u_wr, uc, uslot = decode(u)
        v = u + G
        v_wr, _, vslot = decode(v)

        @pl.when(jnp.logical_not(t_wr))
        def _():
            wait_all(rd(c, slot))

        @pl.when(t_wr)
        def _():
            wait_all(wr(c, slot))

        @pl.when(jnp.logical_and(jnp.logical_not(u_wr), u < n_steps))
        def _():
            rd_start(uc, uslot)

        @pl.when(jnp.logical_and(u_wr, u < n_steps))
        def _():
            wr_start(uc, uslot)

        @pl.when(jnp.logical_not(t_wr))
        def _():
            stats(c, slot)

        @pl.when(jnp.logical_and(v_wr, v < n_steps))
        def _():
            normalise(vslot)

        return carry

    lax.fori_loop(0, n_steps, body, 0)


@jax.jit
def pallas_standalone__instancenorm__prompt_kernel(
    x: jax.Array,
    g: jax.Array,
    b: jax.Array,
):
    B, C, H, W = x.shape
    n_inst = B * C
    bursts = _bursts(n_inst // _R)
    assert min(bursts) >= _D + _G and sum(bursts) * _R == n_inst
    n_slots = max(bursts)
    n_res = n_slots * _R
    view = (_Q, _TILE, H)
    xt = jnp.transpose(x, (0, 1, 3, 2)).reshape(n_inst * W // (_Q * _TILE), *view)
    f32 = jnp.float32
    g_rows = C // _LANES
    out = pl.pallas_call(
        functools.partial(_kernel, bursts=bursts, n_ch=C, rows=W, cols=H),
        in_specs=[pl.BlockSpec(memory_space=pl.ANY)] * 3,
        out_specs=pl.BlockSpec(memory_space=pl.ANY),
        out_shape=jax.ShapeDtypeStruct(xt.shape, x.dtype),
        scratch_shapes=[
            pltpu.VMEM((n_res * W // (_Q * _TILE), *view), x.dtype),
            pltpu.VMEM((_R, _SUB, _LANES), f32),
            pltpu.VMEM((n_res, _SUB, _LANES), f32),
            pltpu.VMEM((n_res, _SUB, _LANES), f32),
            pltpu.VMEM((n_res, _SUB, _LANES), f32),
            pltpu.VMEM((2, g_rows, _LANES), g.dtype),
            pltpu.VMEM((2 * g_rows, _LANES), f32),
            pltpu.SMEM((2 * g_rows, _LANES), f32),
            pltpu.SemaphoreType.DMA((n_slots,)),
            pltpu.SemaphoreType.DMA((2,)),
        ],
        compiler_params=pltpu.CompilerParams(
            vmem_limit_bytes=110 * 1024 * 1024, disable_bounds_checks=True),
    )(xt, g.reshape(g_rows, _LANES), b.reshape(g_rows, _LANES))
    return jnp.transpose(out.reshape(B, C, W, H), (0, 1, 3, 2))
```
